```python
import jax
import jax.numpy as jnp

def _softmax(x, axis=-1):
    return jax.nn.softmax(x, axis=axis)
def _gelu(x):
    return jax.nn.gelu(x, approximate=True)
def _silu(x):
    return jax.nn.silu(x)
def _sigmoid(x):
    return jax.nn.sigmoid(x)
def _layernorm(x, axis=-1, eps=1e-5):
    m = jnp.mean(x, axis=axis, keepdims=True)
    v = jnp.var(x, axis=axis, keepdims=True)
    return (x - m) / jnp.sqrt(v + eps)
def _scatter_add(tgt, idx, src, axis=0):
    return tgt.at[idx].add(src)
def _segment_sum(src, seg, n):
    return jax.ops.segment_sum(src, seg, n)
class _Rng:
    def __init__(self, key):
        self._k = key
    def _next(self):
        self._k, sub = jax.random.split(self._k)
        return sub
    def normal(self, shape):
        return jax.random.normal(self._next(), shape, dtype=jnp.bfloat16)
    def randint(self, lo, hi, shape):
        return jax.random.randint(self._next(), shape, lo, hi, dtype=jnp.int32)
    def uniform(self, shape, lo=0.0, hi=1.0):
        return jax.random.uniform(self._next(), shape, jnp.bfloat16, lo, hi)
    def permutation(self, n):
        return jax.random.permutation(self._next(), n)


kernel_name = 'recurrent_scan__sliding_block_cached__mixer_s_mlp__decode'

def _fwd_setup_inputs():
    _rng = _Rng(jax.random.key(int.from_bytes(__import__("os").urandom(4), "little")))
    _w = (lambda a: (lambda t: t.astype(jnp.bfloat16) if jnp.issubdtype(t.dtype, jnp.floating) else t)(jnp.asarray(a)))
    def _A_setup():
        B, Sq, D = 4, 1, 512
        Hq, Hkv, Sk, Dh = 32, 8, 8192, 128
        assert Hq % Hkv == 0, (Hq, Hkv)
        return {
            "x": _w((lambda *s: _rng.normal(s) * 0.05)(B, Sq, D)),
            "k_cache": _w((lambda *s: _rng.normal(s) * 0.05)(B, Hkv, Sk, Dh)),
            "v_cache": _w((lambda *s: _rng.normal(s) * 0.05)(B, Hkv, Sk, Dh)),
            "wq": _w((lambda *s: _rng.normal(s) * 0.05)(D, Hq * Dh) * (D ** -0.5)),
            "wo": _w((lambda *s: _rng.normal(s) * 0.05)(Hq * Dh, D) * ((Hq * Dh) ** -0.5)),
        }
    _A_in = _A_setup()

    def _B_setup():
        B, S, D, F = 4, 1, 512, 1792
        return {
            "x":  _w((lambda *s: _rng.normal(s) * 0.05)(B, S, D)),
            "w1": _w((lambda *s: _rng.normal(s) * 0.05)(D, D) * (D ** -0.5)),
            "w2": _w((lambda *s: _rng.normal(s) * 0.05)(D, D) * (D ** -0.5)),
            "w3": _w((lambda *s: _rng.normal(s) * 0.05)(D, F) * (D ** -0.5)),
            "w4": _w((lambda *s: _rng.normal(s) * 0.05)(F, D) * (F ** -0.5)),
        }
    _B_in = _B_setup()

    return {
        "A_x": _A_in["x"],
        "A_k_cache": _A_in["k_cache"],
        "A_v_cache": _A_in["v_cache"],
        "A_wq": _A_in["wq"],
        "A_wo": _A_in["wo"],
        "B_x": _B_in["x"],
        "B_w1": _B_in["w1"],
        "B_w2": _B_in["w2"],
        "B_w3": _B_in["w3"],
        "B_w4": _B_in["w4"],
    }

def _fwd_reference(A_x, A_k_cache, A_v_cache, A_wq, A_wo, B_x, B_w1, B_w2, B_w3, B_w4):
    def _A_ref(x, k_cache, v_cache, wq, wo):
        B, Sq, D = x.shape
        Hq, Dh = 32, 128
        Hkv, Sk = k_cache.shape[1], k_cache.shape[2]
        W = min(4096, max(256, Sk // 4))
        rep = Hq // Hkv
        q = (lambda x, *d: x.transpose(*d))((x @ wq).reshape(B, Sq, Hq, Dh), 0, 2, 1, 3)
        k = jnp.repeat(k_cache[:, :, Sk - W:, :], rep, axis=1)
        v = jnp.repeat(v_cache[:, :, Sk - W:, :], rep, axis=1)
        scores = jnp.einsum("bhqd,bhkd->bhqk", q, k) * (Dh ** -0.5)
        p = _softmax(scores, axis=-1)
        o = jnp.einsum("bhqk,bhkd->bhqd", p, v)
        return (lambda x, *d: x.transpose(*d))(o, 0, 2, 1, 3).reshape(B, Sq, Hq * Dh) @ wo

    def _B_ref(x, w1, w2, w3, w4):
        B, S, D = x.shape
        h = _gelu(_layernorm(x, axis=-1) @ w1)
        c = D // 4
        g0 = jnp.pad(h[:, :, 0*c:1*c], ((0, 0), (1, 0), (0, 0)))[:, :S, :]
        g1 = jnp.pad(h[:, :, 1*c:2*c], ((0, 0), (0, 1), (0, 0)))[:, 1:, :]
        g2 = jnp.pad(h[:, :, 2*c:3*c], ((0, 0), (2, 0), (0, 0)))[:, :S, :]
        g3 = jnp.pad(h[:, :, 3*c:   ], ((0, 0), (0, 2), (0, 0)))[:, 2:, :]
        hs = jnp.concatenate([g0, g1, g2, g3], axis=-1) @ w2
        x1 = x + hs
        h2 = _gelu(_layernorm(x1, axis=-1) @ w3) @ w4
        return x1 + h2

    x = A_x
    xn = _layernorm(x, axis=-1)
    s = _A_ref(xn, A_k_cache, A_v_cache, A_wq, A_wo)
    g = _silu(_B_ref(xn, B_w1, B_w2, B_w3, B_w4))
    return x + s * g


def setup_inputs():
    _inp = _fwd_setup_inputs()
    _gk = jax.random.fold_in(jax.random.key(int.from_bytes(__import__("os").urandom(4), "little")), 2**31 - 1)
    _shapes = [[4, 1, 512]]
    _dtypes = ['bfloat16']
    _gks = jax.random.split(_gk, len(_shapes))
    _gs = [jax.random.normal(k, s, dtype=jnp.dtype(d)) * 0.05 for k, s, d in zip(_gks, _shapes, _dtypes)]
    _inp["grad_out"] = _gs[0]
    return _inp

def reference(A_x, A_k_cache, A_v_cache, A_wq, A_wo, B_w3, B_w4, B_x, B_w1, B_w2, grad_out):
    _const = dict(B_x=B_x, B_w1=B_w1, B_w2=B_w2)
    def _f(*_d):
        return _fwd_reference(**{'A_x': _d[0], 'A_k_cache': _d[1], 'A_v_cache': _d[2], 'A_wq': _d[3], 'A_wo': _d[4], 'B_w3': _d[5], 'B_w4': _d[6], **_const})
    _out, _vjp = jax.vjp(_f, A_x, A_k_cache, A_v_cache, A_wq, A_wo, B_w3, B_w4)
    _grads = _vjp(grad_out)
    _out0 = jnp.asarray(_out)
    return (_out0, *[jnp.asarray(_g) for _g in _grads])
```

```python
import functools

import jax
import jax.numpy as jnp
from jax import lax
import jax.experimental.pallas as pl
import jax.experimental.pallas.tpu as pltpu

F32 = jnp.float32
BF16 = jnp.bfloat16

HQ = 32
DH = 128
EPS = 1e-5
SQRT_2_OVER_PI = 0.7978845608028654
GELU_C = 0.044715

NN = (((1,), (0,)), ((), ()))
NT = (((1,), (1,)), ((), ()))
TN = (((0,), (0,)), ((), ()))


def _dot(a, b, dims):
    return lax.dot_general(a, b, dims, preferred_element_type=F32)


def _ln_fwd(x):
    m = jnp.mean(x, axis=-1, keepdims=True)
    xc = x - m
    v = jnp.mean(xc * xc, axis=-1, keepdims=True)
    r = 1.0 / jnp.sqrt(v + EPS)
    return xc * r, r


def _ln_bwd(y, r, dy):
    return r * (dy - jnp.mean(dy, axis=-1, keepdims=True)
                - y * jnp.mean(dy * y, axis=-1, keepdims=True))


def _loop(n, body, unroll=1):
    def wrapped(i, c):
        for u in range(unroll):
            body(i * unroll + u)
        return c
    assert n % unroll == 0
    lax.fori_loop(0, n // unroll, wrapped, 0)


def make(cfg=None):
    cfg = dict(cfg or {})
    RR = cfg.get("rr", 16)
    WR = cfg.get("wr", 64)
    NZ0 = cfg.get("nz0", 48)
    compute = cfg.get("compute", True)

    def kernel(x_hbm, k_hbm, v_hbm, wq_hbm, wo_hbm, w3_hbm, w4_hbm, do_hbm,
               out_hbm, dx_hbm, dk_hbm, dv_hbm, dwq_hbm, dwo_hbm, dw3_hbm, dw4_hbm,
               x_v, go_v, k_v, v_v, wq_v, wo_v, w3_v, w4_v,
               out_v, dx_v, dk_v, dv_v, dwq_v, dwo_v, dw3_v, dw4_v,
               zero_v, q2, do2, o2, dq2, rsem, wsem):
        B, HKV, SK, _ = k_hbm.shape
        W = k_v.shape[2]
        ZR = SK - W
        D = wq_hbm.shape[0]
        F = w3_hbm.shape[1]
        REP = HQ // HKV
        scale = DH ** -0.5

        pltpu.make_async_copy(x_hbm, x_v, rsem.at[0]).start()
        pltpu.make_async_copy(do_hbm, go_v, rsem.at[1]).start()

        rnc = W // RR

        def rd_kv(i):
            b = i // rnc
            c = i % rnc
            r0 = pl.multiple_of(c * RR, RR)
            pltpu.make_async_copy(k_hbm.at[b, :, pl.ds(ZR + r0, RR)],
                                  k_v.at[b, :, pl.ds(r0, RR)], rsem.at[2]).start(priority=0)
            pltpu.make_async_copy(v_hbm.at[b, :, pl.ds(ZR + r0, RR)],
                                  v_v.at[b, :, pl.ds(r0, RR)], rsem.at[3]).start(priority=1)

        def rd_w(a_hbm, a_v, sa, b_hbm, b_v, sb, n):
            def body(i):
                r0 = pl.multiple_of((i % 4) * 128, 128)
                c0 = pl.multiple_of((i // 4) * 128, 128)
                pltpu.make_async_copy(a_hbm.at[pl.ds(r0, 128), pl.ds(c0, 128)],
                                      a_v.at[pl.ds(r0, 128), pl.ds(c0, 128)], rsem.at[sa]).start(priority=0)
                j = (i % 4) * (n // 4) + i // 4
                s0 = pl.multiple_of(j * 32, 32)
                pltpu.make_async_copy(b_hbm.at[pl.ds(s0, 32)], b_v.at[pl.ds(s0, 32)], rsem.at[sb]).start(priority=1)
            _loop(n, body, unroll=2)

        rd_w(wq_hbm, wq_v, 4, wo_hbm, wo_v, 5, HQ * DH // 32)
        zero_v[...] = jnp.zeros(zero_v.shape, zero_v.dtype)
        rd_w(w3_hbm, w3_v, 6, w4_hbm, w4_v, 7, F // 32)
        _loop(B * rnc, rd_kv, unroll=2)

        for ref, s in ((x_v, 0), (go_v, 1), (wq_v, 4), (wo_v, 5), (w3_v, 6), (w4_v, 7), (k_v, 2), (v_v, 3)):
            pltpu.make_async_copy(ref, ref, rsem.at[s]).wait()

        znc = ZR // WR
        NZ = 2 * B * znc

        def wr_zero(i):
            t = i // (B * znc)
            j = i % (B * znc)
            b = j // znc
            r0 = pl.multiple_of((j % znc) * WR, WR)

            @pl.when(t == 0)
            def _():
                pltpu.make_async_copy(zero_v, dk_hbm.at[b, :, pl.ds(r0, WR)], wsem.at[2]).start()

            @pl.when(t == 1)
            def _():
                pltpu.make_async_copy(zero_v, dv_hbm.at[b, :, pl.ds(r0, WR)], wsem.at[3]).start()

        def zeros(lo, n):
            _loop(n, lambda i: wr_zero(lo + i))

        n_first = 2 * NZ0
        zeros(0, n_first)

        pad = jnp.zeros((8 - B, D), F32)
        x = jnp.concatenate([x_v[...].astype(F32), pad], axis=0)
        go = jnp.concatenate([go_v[...].astype(F32), pad], axis=0)
        xn, r0_ = _ln_fwd(x)
        u, r1_ = _ln_fwd(xn)
        xn_b = xn.astype(BF16)
        u_b = u.astype(BF16)
        pre = _dot(u_b, w3_v[...], NN)
        inner = SQRT_2_OVER_PI * (pre + GELU_C * pre * pre * pre)
        th = jnp.tanh(inner)
        a = 0.5 * pre * (1.0 + th)
        dgelu = 0.5 * (1.0 + th) + 0.5 * pre * (1.0 - th * th) * SQRT_2_OVER_PI * (1.0 + 3.0 * GELU_C * pre * pre)
        a_b = a.astype(BF16)
        y = xn + _dot(a_b, w4_v[...], NN)
        sig = jax.nn.sigmoid(y)
        g = y * sig
        ds = go * g
        ds_b = ds.astype(BF16)
        q = _dot(xn_b, wq_v[...], NN)
        dar = _dot(ds_b, wo_v[...], NT)
        for h in range(HQ):
            q2[pl.ds(h, B, stride=HQ), :] = q[0:B, h * DH:(h + 1) * DH]
            do2[pl.ds(h, B, stride=HQ), :] = dar[0:B, h * DH:(h + 1) * DH]

        n_it = B * HKV // 2
        per_it = (NZ - n_first) // n_it
        assert per_it * n_it == NZ - n_first
        lo = lax.broadcasted_iota(jnp.int32, (8, 1), 0) < REP

        def attn(i):
            zeros(n_first + i * per_it, per_it)
            if not compute:
                return
            b = i // (HKV // 2)
            g0 = (i % (HKV // 2)) * 2
            r = pl.multiple_of(i * 8, 8)
            qf = q2[pl.ds(r, 8), :]
            dof = do2[pl.ds(r, 8), :]
            q8 = qf.astype(BF16)
            do8 = dof.astype(BF16)
            s = jnp.where(lo, _dot(q8, k_v[b, g0], NT), _dot(q8, k_v[b, g0 + 1], NT)) * scale
            m = jnp.max(s, axis=-1, keepdims=True)
            e = jnp.exp(s - m)
            p = e * (1.0 / jnp.sum(e, axis=-1, keepdims=True))
            dp = jnp.where(lo, _dot(do8, v_v[b, g0], NT), _dot(do8, v_v[b, g0 + 1], NT))
            dsc = p * (dp - jnp.sum(p * dp, axis=-1, keepdims=True)) * scale
            p_b = p.astype(BF16)
            dsc_b = dsc.astype(BF16)
            o2[pl.ds(r, 8), :] = jnp.where(lo, _dot(p_b, v_v[b, g0], NN), _dot(p_b, v_v[b, g0 + 1], NN))
            dq2[pl.ds(r, 8), :] = jnp.where(lo, _dot(dsc_b, k_v[b, g0], NN), _dot(dsc_b, k_v[b, g0 + 1], NN))
            lhs = jnp.concatenate([p, dsc], axis=0).astype(BF16)
            z = jnp.zeros((8, DH), F32)
            rhs = jnp.concatenate([
                jnp.concatenate([jnp.where(lo, dof, 0.0), jnp.where(lo, 0.0, dof), z, z], axis=1),
                jnp.concatenate([z, z, jnp.where(lo, qf, 0.0), jnp.where(lo, 0.0, qf)], axis=1),
            ], axis=0).astype(BF16)
            CH = 512
            for c in range(W // CH):
                res = _dot(lhs[:, c * CH:(c + 1) * CH], rhs, TN).astype(BF16)
                dv_v[b, g0, pl.ds(c * CH, CH), :] = res[:, 0:DH]
                dv_v[b, g0 + 1, pl.ds(c * CH, CH), :] = res[:, DH:2 * DH]
                dk_v[b, g0, pl.ds(c * CH, CH), :] = res[:, 2 * DH:3 * DH]
                dk_v[b, g0 + 1, pl.ds(c * CH, CH), :] = res[:, 3 * DH:4 * DH]

        _loop(n_it, attn)

        dnc = W // WR

        def wr_kv(src, dst, sem, j):
            b = j // dnc
            r0 = pl.multiple_of((j % dnc) * WR, WR)
            pltpu.make_async_copy(src.at[b, :, pl.ds(r0, WR)], dst.at[b, :, pl.ds(ZR + r0, WR)], wsem.at[sem]).start()

        half = B * dnc // 2
        _loop(half, lambda j: wr_kv(dk_v, dk_hbm, 2, j))

        pad4 = jnp.zeros((8 - B, DH), F32)
        o_b = jnp.concatenate(
            [jnp.concatenate([o2[pl.ds(h, B, stride=HQ), :], pad4], axis=0) for h in range(HQ)], axis=1).astype(BF16)
        dq_b = jnp.concatenate(
            [jnp.concatenate([dq2[pl.ds(h, B, stride=HQ), :], pad4], axis=0) for h in range(HQ)], axis=1).astype(BF16)
        s_att = _dot(o_b, wo_v[...], NN)
        out = x + s_att * g
        dy = go * s_att * (sig * (1.0 + y * (1.0 - sig)))
        dy_b = dy.astype(BF16)
        dpre = _dot(dy_b, w4_v[...], NT) * dgelu
        dpre_b = dpre.astype(BF16)
        du = _dot(dpre_b, w3_v[...], NT)
        dxn = _dot(dq_b, wq_v[...], NT) + dy + _ln_bwd(u, r1_, du)
        dx = go + _ln_bwd(xn, r0_, dxn)
        out_v[...] = out[0:B].astype(BF16)
        dx_v[...] = dx[0:B].astype(BF16)
        pltpu.make_async_copy(out_v, out_hbm, wsem.at[0]).start()
        pltpu.make_async_copy(dx_v, dx_hbm, wsem.at[1]).start()

        _loop(half, lambda j: wr_kv(dk_v, dk_hbm, 2, half + j))
        for c in range(HQ * DH // 512):
            sl = slice(c * 512, (c + 1) * 512)
            dwq_v[:, sl] = _dot(xn_b, dq_b[:, sl], TN).astype(BF16)
            dwo_v[sl, :] = _dot(o_b[:, sl], ds_b, TN).astype(BF16)
        _loop(half, lambda j: wr_kv(dv_v, dv_hbm, 3, j))
        for c in range(F // 256):
            sl = slice(c * 256, (c + 1) * 256)
            dw3_v[:, sl] = _dot(u_b, dpre_b[:, sl], TN).astype(BF16)
            dw4_v[sl, :] = _dot(a_b[:, sl], dy_b, TN).astype(BF16)
        _loop(half, lambda j: wr_kv(dv_v, dv_hbm, 3, half + j))

        def wr_w(a_v, a_hbm, sa, b_v, b_hbm, sb, n):
            def body(i):
                r0 = pl.multiple_of((i % 4) * 128, 128)
                c0 = pl.multiple_of((i // 4) * 128, 128)
                pltpu.make_async_copy(a_v.at[pl.ds(r0, 128), pl.ds(c0, 128)],
                                      a_hbm.at[pl.ds(r0, 128), pl.ds(c0, 128)], wsem.at[sa]).start()
                j = (i % 4) * (n // 4) + i // 4
                s0 = pl.multiple_of(j * 32, 32)
                pltpu.make_async_copy(b_v.at[pl.ds(s0, 32)], b_hbm.at[pl.ds(s0, 32)], wsem.at[sb]).start()
            _loop(n, body, unroll=2)

        wr_w(dwq_v, dwq_hbm, 4, dwo_v, dwo_hbm, 5, HQ * DH // 32)
        wr_w(dw3_v, dw3_hbm, 6, dw4_v, dw4_hbm, 7, F // 32)

        for ref, s in ((out_hbm, 0), (dx_hbm, 1), (dk_hbm, 2), (dv_hbm, 3),
                       (dwq_hbm, 4), (dwo_hbm, 5), (dw3_hbm, 6), (dw4_hbm, 7)):
            pltpu.make_async_copy(ref, ref, wsem.at[s]).wait()

    def fn(A_x, A_k_cache, A_v_cache, A_wq, A_wo, B_x, B_w1, B_w2, B_w3, B_w4, grad_out):
        del B_x, B_w1, B_w2
        B, HKV, SK, _ = A_k_cache.shape
        W = min(4096, max(256, SK // 4))
        hbm = pl.BlockSpec(memory_space=pltpu.HBM)
        x_shape = A_x.shape
        A_x = A_x.reshape(B, -1)
        grad_out = grad_out.reshape(B, -1)
        ins = (A_x, A_k_cache, A_v_cache, A_wq, A_wo, B_w3, B_w4, grad_out)
        outs = (A_x, A_x, A_k_cache, A_v_cache, A_wq, A_wo, B_w3, B_w4)
        vm = lambda a: pltpu.VMEM(a.shape, a.dtype)
        win = pltpu.VMEM((B, HKV, W, DH), BF16)
        small = pltpu.VMEM((B * HQ, DH), F32)
        res = pl.pallas_call(
            kernel,
            out_shape=[jax.ShapeDtypeStruct(a.shape, a.dtype) for a in outs],
            in_specs=[hbm] * len(ins),
            out_specs=[hbm] * len(outs),
            scratch_shapes=[
                vm(A_x), vm(grad_out), win, win, vm(A_wq), vm(A_wo), vm(B_w3), vm(B_w4),
                vm(A_x), vm(A_x), win, win, vm(A_wq), vm(A_wo), vm(B_w3), vm(B_w4),
                pltpu.VMEM((HKV, WR, DH), BF16), small, small, small, small,
                pltpu.SemaphoreType.DMA((8,)), pltpu.SemaphoreType.DMA((8,)),
            ],
            compiler_params=pltpu.CompilerParams(vmem_limit_bytes=120 * 1024 * 1024),
        )(*ins)
        return (res[0].reshape(x_shape), res[1].reshape(x_shape), *res[2:])

    return fn


_impl = make()


@jax.jit
def pallas_recurrent_scan__sliding_block_cached__mixer_s_mlp__decode_kernel(
        A_x, A_k_cache, A_v_cache, A_wq, A_wo, B_x, B_w1, B_w2, B_w3, B_w4, grad_out):
    return tuple(_impl(A_x, A_k_cache, A_v_cache, A_wq, A_wo, B_x, B_w1, B_w2, B_w3, B_w4, grad_out))
```

```python
import jax
import jax.numpy as jnp
from jax import lax
import jax.experimental.pallas as pl
import jax.experimental.pallas.tpu as pltpu

F32 = jnp.float32
BF16 = jnp.bfloat16

HQ = 32
DH = 128
EPS = 1e-5
SQRT_2_OVER_PI = 0.7978845608028654
GELU_C = 0.044715

NN = (((1,), (0,)), ((), ()))
NT = (((1,), (1,)), ((), ()))
TN = (((0,), (0,)), ((), ()))


def _dot(a, b, dims):
    return lax.dot_general(a, b, dims, preferred_element_type=F32)


def _ln_fwd(x):
    m = jnp.mean(x, axis=-1, keepdims=True)
    xc = x - m
    v = jnp.mean(xc * xc, axis=-1, keepdims=True)
    r = 1.0 / jnp.sqrt(v + EPS)
    return xc * r, r


def _ln_bwd(y, r, dy):
    return r * (dy - jnp.mean(dy, axis=-1, keepdims=True)
                - y * jnp.mean(dy * y, axis=-1, keepdims=True))


def _loop(n, body, unroll=1):
    assert n % unroll == 0, (n, unroll)
    if n == unroll:
        for u in range(n):
            body(u)
        return

    def wrapped(i, c):
        for u in range(unroll):
            body(i * unroll + u)
        return c
    if n:
        lax.fori_loop(0, n // unroll, wrapped, 0)


def _ds(start, size, align):
    if not isinstance(start, int):
        start = pl.multiple_of(start, align)
    return pl.ds(start, size)


def _start(src, dst, sem, priority=0):
    pltpu.make_async_copy(src, dst, sem).start(priority=priority)


def _wait(ref, sem):
    pltpu.make_async_copy(ref, ref, sem).wait()


def _copy_slab_rows(src, dst, i, rows, cols, sem, priority=0):
    r = _ds(i * rows, rows, rows)
    for c in range(0, src.shape[2], cols):
        _start(src.at[:, r, pl.ds(c, cols)], dst.at[:, r, pl.ds(c, cols)], sem, priority)


def make(cfg=None):
    cfg = dict(cfg or {})
    RR = cfg.get("rr", 16)
    RS = cfg.get("rs", 8)
    TAIL = cfg.get("tail", 64)
    WA = cfg.get("wa", 16)
    WB = cfg.get("wb", 16)
    UA = cfg.get("ua", 8)
    UB = cfg.get("ub", 8)
    compute = cfg.get("compute", True)
    cparams = cfg.get("cparams", {})
    w_pos = cfg.get("w_pos", "mid")
    HU = 3

    def kernel(x_hbm, k_hbm, v_hbm, wq_hbm, wo_hbm, w3_hbm, w4_hbm, go_hbm,
               out_hbm, dx_hbm, dk_hbm, dv_hbm, dwq_hbm, dwo_hbm, dw3_hbm, dw4_hbm,
               x_v, go_v, k_v, v_v, wq_v, wo_v, w3_v, w4_v,
               out_v, dx_v, dk_v, dv_v, dwq_v, dwo_v, dw3_v, dw4_v,
               zero_v, q_s, do_s, o_s, dq_s, kv_sem):
        B, D = x_v.shape
        BH, W, _ = k_v.shape
        HKV = BH // B
        ZR = k_hbm.shape[1] - W
        F = w3_v.shape[2]
        REP = HQ // HKV
        scale = DH ** -0.5
        CH = 512
        UNITS = BH // HU
        REST = BH - UNITS * HU
        grads = ((dk_hbm, dk_v), (dv_hbm, dv_v))

        def zero_fill(unit, part, parts):
            n = W // WA // parts
            for t, (o, _) in enumerate(grads):
                def go(t=t, o=o):
                    heads = pl.ds((unit - t * UNITS) * HU, HU)
                    _loop(n, lambda c: _start(
                        zero_v.at[pl.ds(0, HU), :, pl.ds(0, WA)],
                        o.at[heads, :, _ds((part * n + c) * WA, WA, WA)], kv_sem.at[t]), min(UA, n))
                if isinstance(unit, int):
                    if unit // UNITS == t:
                        go()
                else:
                    pl.when((unit >= UNITS) if t else (unit < UNITS))(go)

        def read_phase(sem):
            def rd_qo(i):
                r = _ds(i * 8, 8, 8)
                for c in range(8):
                    _start(wq_hbm.at[:, r, pl.ds(c * 512, 512)], wq_v.at[:, r, pl.ds(c * 512, 512)], sem.at[2], 0)
                    _copy_slab_rows(wo_hbm, wo_v, i * 8 + c, 8, D, sem.at[3], 1)
            _loop(wq_v.shape[1] // 8, rd_qo)
            _start(x_hbm, x_v, sem.at[0])
            _start(go_hbm, go_v, sem.at[1], 1)
            zero_v[...] = jnp.zeros(zero_v.shape, zero_v.dtype)
            o_s[...] = jnp.zeros(o_s.shape, o_s.dtype)
            dq_s[...] = jnp.zeros(dq_s.shape, dq_s.dtype)

            def rd_34(i):
                r = _ds(i * 8, 8, 8)
                for c in range(2):
                    cs = pl.ds(c * (F // 2), F // 2)
                    _start(w3_hbm.at[:, r, cs], w3_v.at[:, r, cs], sem.at[4], 0)
                    pl.when(i * 2 + c < w4_v.shape[1] // 16)(
                        lambda c=c: _copy_slab_rows(w4_hbm, w4_v, i * 2 + c, 16, D, sem.at[5], 1))
            _loop(w3_v.shape[1] // 8, rd_34)

            def rd_kv(lo, rows, sk, sv):
                def group(g):
                    heads = pl.ds(g * RS, RS)

                    def chunk(c):
                        src = (heads, _ds(ZR + lo + c * RR, RR, RR))
                        dst = (heads, _ds(lo + c * RR, RR, RR))
                        _start(k_hbm.at[src], k_v.at[dst], sem.at[sk], 0)
                        _start(v_hbm.at[src], v_v.at[dst], sem.at[sv], 1)
                    _loop(rows // RR, chunk, 4 if (rows // RR) % 4 == 0 else 1)
                _loop(BH // RS, group)
            rd_kv(0, W - TAIL, 6, 7)
            rd_kv(W - TAIL, TAIL, 8, 9)

            for s, ref in enumerate((x_v, go_v, wq_v, wo_v, w3_v, w4_v)):
                _wait(ref, sem.at[s])
            _wait(k_v.at[:, pl.ds(0, W - TAIL)], sem.at[6])
            _wait(v_v.at[:, pl.ds(0, W - TAIL)], sem.at[7])
            zero_fill(16, 0, 1)
            _wait(k_v.at[:, pl.ds(W - TAIL, TAIL)], sem.at[8])
            _wait(v_v.at[:, pl.ds(W - TAIL, TAIL)], sem.at[9])

        pl.run_scoped(read_phase, pltpu.SemaphoreType.DMA((10,)))

        pad = jnp.zeros((8 - B, D), F32)
        x = jnp.concatenate([x_v[...].astype(F32), pad], axis=0)
        go = jnp.concatenate([go_v[...].astype(F32), pad], axis=0)
        xn, r0_ = _ln_fwd(x)
        u, r1_ = _ln_fwd(xn)
        xn_b = xn.astype(BF16)
        u_b = u.astype(BF16)
        pre = _dot(u_b, w3_v[...].reshape(D, F), NN)
        inner = SQRT_2_OVER_PI * (pre + GELU_C * pre * pre * pre)
        th = jnp.tanh(inner)
        a = 0.5 * pre * (1.0 + th)
        dgelu = 0.5 * (1.0 + th) + 0.5 * pre * (1.0 - th * th) * SQRT_2_OVER_PI * (1.0 + 3.0 * GELU_C * pre * pre)
        a_b = a.astype(BF16)
        y = xn + _dot(a_b, w4_v[...].reshape(F, D), NN)
        sig = jax.nn.sigmoid(y)
        g = y * sig
        ds_b = (go * g).astype(BF16)

        zero_fill(17, 0, 2)

        hpc = CH // DH
        n_ch = HQ // hpc
        wo_n = wo_v.shape[1] // CH

        def wq_chunk(c):
            return wq_v[:, :, _ds(c * CH, CH, CH)].reshape(D, CH)

        def wo_rows(c):
            return lax.div(c, wo_n), _ds(lax.rem(c, wo_n) * CH, CH, CH)

        def proj(c):
            zero_fill(17, n_ch + c, 2 * n_ch)
            q = _dot(xn_b, wq_chunk(c), NN)
            do = _dot(ds_b, wo_v[wo_rows(c)], NT)
            for i in range(hpc):
                r = _ds((c * hpc + i) * 8, 8, 8)
                q_s[r, :] = q[:, i * DH:(i + 1) * DH]
                do_s[r, :] = do[:, i * DH:(i + 1) * DH]

        _loop(n_ch, proj)

        lo = lax.broadcasted_iota(jnp.int32, (8, 1), 0) < REP

        def attn(i):
            zero_fill(i, 0, 2)
            if not compute:
                zero_fill(i, 1, 2)
                return
            j = 2 * i
            rows = pl.ds(lax.rem(i, HKV // 2) * 64 + lax.div(i, HKV // 2), 8, stride=8)
            qf = q_s[rows, :]
            dof = do_s[rows, :]
            q8 = qf.astype(BF16)
            do8 = dof.astype(BF16)
            s = jnp.where(lo, _dot(q8, k_v[j], NT), _dot(q8, k_v[j + 1], NT)) * scale
            m = jnp.max(s, axis=-1, keepdims=True)
            e = jnp.exp(s - m)
            p = e * (1.0 / jnp.sum(e, axis=-1, keepdims=True))
            dp = jnp.where(lo, _dot(do8, v_v[j], NT), _dot(do8, v_v[j + 1], NT))
            dsc = p * (dp - jnp.sum(p * dp, axis=-1, keepdims=True)) * scale
            p_b = p.astype(BF16)
            dsc_b = dsc.astype(BF16)
            o_s[rows, :] = jnp.where(lo, _dot(p_b, v_v[j], NN), _dot(p_b, v_v[j + 1], NN))
            dq_s[rows, :] = jnp.where(lo, _dot(dsc_b, k_v[j], NN), _dot(dsc_b, k_v[j + 1], NN))
            zero_fill(i, 1, 2)
            lhs = jnp.concatenate([p, dsc], axis=0).astype(BF16)
            z = jnp.zeros((8, DH), F32)
            rhs = jnp.concatenate([
                jnp.concatenate([jnp.where(lo, dof, 0.0), jnp.where(lo, 0.0, dof), z, z], axis=1),
                jnp.concatenate([z, z, jnp.where(lo, qf, 0.0), jnp.where(lo, 0.0, qf)], axis=1),
            ], axis=0).astype(BF16)
            for c in range(W // CH):
                sl = pl.ds(c * CH, CH)
                res = _dot(lhs[:, c * CH:(c + 1) * CH], rhs, TN).astype(BF16)
                dv_v[j, sl, :] = res[:, 0:DH]
                dv_v[j + 1, sl, :] = res[:, DH:2 * DH]
                dk_v[j, sl, :] = res[:, 2 * DH:3 * DH]
                dk_v[j + 1, sl, :] = res[:, 3 * DH:4 * DH]

        _loop(BH // 2, attn)

        def proj_bwd(c, carry):
            s_att, dxn = carry
            zero_fill(18 + lax.div(c, n_ch // 2), lax.rem(c, n_ch // 2), n_ch // 2)
            heads = [_ds((c * hpc + i) * 8, 8, 8) for i in range(hpc)]
            o_c = jnp.concatenate([o_s[r, :] for r in heads], axis=1).astype(BF16)
            dq_c = jnp.concatenate([dq_s[r, :] for r in heads], axis=1).astype(BF16)
            s_att += _dot(o_c, wo_v[wo_rows(c)], NN)
            dxn += _dot(dq_c, wq_chunk(c), NT)
            dwq_v[:, :, _ds(c * CH, CH, CH)] = _dot(xn_b, dq_c, TN).astype(BF16).reshape(dwq_v.shape[0], -1, CH)
            dwo_v[wo_rows(c)] = _dot(o_c, ds_b, TN).astype(BF16)
            return s_att, dxn

        s_att, dxn = lax.fori_loop(0, n_ch, proj_bwd, (jnp.zeros((8, D), F32), jnp.zeros((8, D), F32)))

        def zero_fill_rest(part, parts):
            n = W // WA // parts

            def body(c):
                for t, (o, _) in enumerate(grads):
                    _start(zero_v.at[pl.ds(0, REST), :, pl.ds(0, WA)],
                           o.at[pl.ds(BH - REST, REST), :, _ds((part * n + c) * WA, WA, WA)], kv_sem.at[t])
            _loop(n, body, min(4, n))

        zero_fill_rest(0, 2)

        out = x + s_att * g
        dy = go * s_att * (sig * (1.0 + y * (1.0 - sig)))
        dy_b = dy.astype(BF16)
        dpre_b = (_dot(dy_b, w4_v[...].reshape(F, D), NT) * dgelu).astype(BF16)
        du = _dot(dpre_b, w3_v[...].reshape(D, F), NT)
        dxn = dxn + dy + _ln_bwd(u, r1_, du)
        dx = go + _ln_bwd(xn, r0_, dxn)
        out_v[...] = out[0:B].astype(BF16)
        dx_v[...] = dx[0:B].astype(BF16)

        zero_fill_rest(1, 2)

        FH = F // dw4_v.shape[0]
        for c in range(dw4_v.shape[0]):
            sl = slice(c * FH, (c + 1) * FH)
            dw3_v[:, :, sl] = _dot(u_b, dpre_b[:, sl], TN).astype(BF16).reshape(dw3_v.shape[0], -1, FH)
            dw4_v[c] = _dot(a_b[:, sl], dy_b, TN).astype(BF16)

        def data_fill(ts, h0, S):
            heads = pl.ds(h0, S)

            def body(c):
                r = _ds(W + c * WB, WB, WB)
                for t in ts:
                    o, src = grads[t]
                    _start(zero_v.at[pl.ds(0, S), 0, pl.ds(0, WB)], o.at[heads, 0, r], kv_sem.at[t])
                    _start(src.at[heads, _ds(c * WB, WB, WB)], o.at[heads, 1, r], kv_sem.at[t])
            _loop(W // WB, body, UB // len(ts))

        def small_writes(sem):
            def wr_q4(i):
                r = _ds(i * 8, 8, 8)
                for c in range(4):
                    cs = pl.ds(c * 1024, 1024)
                    _start(dwq_v.at[:, r, cs], dwq_hbm.at[:, r, cs], sem.at[2])
                    pl.when(i * 4 + c < dw4_v.shape[1] // 16)(
                        lambda c=c: _copy_slab_rows(dw4_v, dw4_hbm, i * 4 + c, 16, D, sem.at[5]))

            def wr_o3(i):
                r = _ds(i * 8, 8, 8)
                for c in range(2):
                    cs = pl.ds(c * (F // 2), F // 2)
                    _copy_slab_rows(dwo_v, dwo_hbm, i * 2 + c, 16, D, sem.at[3])
                    _start(dw3_v.at[:, r, cs], dw3_hbm.at[:, r, cs], sem.at[4])

            def all_w():
                _start(out_v, out_hbm, sem.at[0])
                _start(dx_v, dx_hbm, sem.at[1])
                _loop(dwq_v.shape[1] // 8, wr_q4)
                _loop(dw3_v.shape[1] // 8, wr_o3)
            if w_pos == "mid":
                all_w()
            data_fill((0, 1), BH - REST, REST)
            _loop(UNITS, lambda i: data_fill((0,), i * HU, HU))
            if w_pos == "late":
                all_w()
            _loop(UNITS, lambda i: data_fill((1,), i * HU, HU))
            for s, ref in enumerate((out_hbm, dx_hbm, dwq_hbm, dwo_hbm, dw3_hbm, dw4_hbm)):
                _wait(ref, sem.at[s])

        pl.run_scoped(small_writes, pltpu.SemaphoreType.DMA((6,)))
        _wait(dk_hbm, kv_sem.at[0])
        _wait(dv_hbm, kv_sem.at[1])

    def fn(A_x, A_k_cache, A_v_cache, A_wq, A_wo, B_x, B_w1, B_w2, B_w3, B_w4, grad_out):
        del B_x, B_w1, B_w2
        B, HKV, SK, _ = A_k_cache.shape
        W = min(4096, max(256, SK // 4))
        assert SK == 4 * W
        like = (A_x, A_x, A_k_cache, A_v_cache, A_wq, A_wo, B_w3, B_w4)
        x = A_x.reshape(B, -1)
        go = grad_out.reshape(B, -1)
        k = A_k_cache.reshape(B * HKV, SK, DH)
        v = A_v_cache.reshape(B * HKV, SK, DH)
        slabs = lambda a, n: a.reshape(n, a.shape[0] // n, a.shape[1])
        wq, wo, w3, w4 = slabs(A_wq, 4), slabs(A_wo, 4), slabs(B_w3, 2), slabs(B_w4, 2)
        dkv = jax.ShapeDtypeStruct((B * HKV, 2, SK // 2, DH), BF16)
        ins = (x, k, v, wq, wo, w3, w4, go)
        outs = (x, x, dkv, dkv, wq, wo, w3, w4)
        hbm = pl.BlockSpec(memory_space=pltpu.HBM)
        vm = lambda a: pltpu.VMEM(a.shape, a.dtype)
        win = pltpu.VMEM((B * HKV, W, DH), BF16)
        small = pltpu.VMEM((HQ * 8, DH), F32)
        res = pl.pallas_call(
            kernel,
            out_shape=[jax.ShapeDtypeStruct(a.shape, a.dtype) for a in outs],
            in_specs=[hbm] * len(ins),
            out_specs=[hbm] * len(outs),
            scratch_shapes=[
                vm(x), vm(go), win, win, vm(wq), vm(wo), vm(w3), vm(w4),
                vm(x), vm(x), win, win, vm(wq), vm(wo), vm(w3), vm(w4),
                pltpu.VMEM((HU, 2, max(WA, WB), DH), BF16), small, small, small, small,
                pltpu.SemaphoreType.DMA((2,)),
            ],
            compiler_params=pltpu.CompilerParams(vmem_limit_bytes=120 * 1024 * 1024, **cparams),
        )(*ins)
        return tuple(r.reshape(a.shape) for r, a in zip(res, like))

    return fn


_impl = make({'wa': 32, 'tail': 48})


@jax.jit
def pallas_recurrent_scan__sliding_block_cached__mixer_s_mlp__decode_kernel(
        A_x, A_k_cache, A_v_cache, A_wq, A_wo, B_x, B_w1, B_w2, B_w3, B_w4, grad_out):
    return _impl(A_x, A_k_cache, A_v_cache, A_wq, A_wo, B_x, B_w1, B_w2, B_w3, B_w4, grad_out)
```

```python
import jax
import jax.numpy as jnp
from jax import lax
import jax.experimental.pallas as pl
import jax.experimental.pallas.tpu as pltpu

F32 = jnp.float32
BF16 = jnp.bfloat16

HQ = 32
DH = 128
EPS = 1e-5
SQRT_2_OVER_PI = 0.7978845608028654
GELU_C = 0.044715

ROWS = 8
CH = 512
READ_HEADS = 8
READ_ROWS = 16
TAIL_ROWS = 48
UNIT_HEADS = 3
ZERO_ROWS = 32
DATA_ROWS = 16

NN = (((1,), (0,)), ((), ()))
NT = (((1,), (1,)), ((), ()))
TN = (((0,), (0,)), ((), ()))


def _dot(a, b, dims):
    return lax.dot_general(a, b, dims, preferred_element_type=F32)


def _layernorm(x):
    xc = x - jnp.mean(x, axis=-1, keepdims=True)
    r = 1.0 / jnp.sqrt(jnp.mean(xc * xc, axis=-1, keepdims=True) + EPS)
    return xc * r, r


def _layernorm_bwd(y, r, dy):
    return r * (dy - jnp.mean(dy, axis=-1, keepdims=True)
                - y * jnp.mean(dy * y, axis=-1, keepdims=True))


def _loop(n, body, unroll=1):
    unroll = min(unroll, n)
    assert n % unroll == 0, (n, unroll)
    if n == unroll:
        for u in range(n):
            body(u)
        return

    def step(i, carry):
        for u in range(unroll):
            body(i * unroll + u)
        return carry

    lax.fori_loop(0, n // unroll, step, 0)


def _ds(start, size, align):
    if not isinstance(start, int):
        start = pl.multiple_of(start, align)
    return pl.ds(start, size)


def _start(src, dst, sem, priority=0):
    pltpu.make_async_copy(src, dst, sem).start(priority=priority)


def _wait(ref, sem):
    pltpu.make_async_copy(ref, ref, sem).wait()


def _copy_rows(src, dst, i, rows, sem, priority=0):
    r = _ds(i * rows, rows, rows)
    _start(src.at[:, r], dst.at[:, r], sem, priority)


def _kernel(x_hbm, k_hbm, v_hbm, wq_hbm, wo_hbm, w3_hbm, w4_hbm, go_hbm,
            out_hbm, dx_hbm, dk_hbm, dv_hbm, dwq_hbm, dwo_hbm, dw3_hbm, dw4_hbm,
            x_v, go_v, k_v, v_v, wq_v, wo_v, w3_v, w4_v,
            out_v, dx_v, dk_v, dv_v, dwq_v, dwo_v, dw3_v, dw4_v,
            zero_v, q_s, do_s, o_s, dq_s, kv_sem):
    batch, d_model = x_v.shape
    n_kv, window, _ = k_v.shape
    kv_heads = n_kv // batch
    first = k_hbm.shape[1] - window
    d_ff = w3_v.shape[2]
    rep = HQ // kv_heads
    scale = DH ** -0.5
    units = n_kv // UNIT_HEADS
    rest = n_kv - units * UNIT_HEADS
    grads = ((dk_hbm, dk_v), (dv_hbm, dv_v))

    def zero_unit(unit, part, parts):
        n = window // ZERO_ROWS // parts
        for t, (grad_hbm, _) in enumerate(grads):
            def issue(t=t, grad_hbm=grad_hbm):
                heads = pl.ds((unit - t * units) * UNIT_HEADS, UNIT_HEADS)
                _loop(n, lambda c: _start(
                    zero_v,
                    grad_hbm.at[heads, :, _ds((part * n + c) * ZERO_ROWS, ZERO_ROWS, ZERO_ROWS)],
                    kv_sem.at[t]), unroll=8)
            if isinstance(unit, int):
                if unit // units == t:
                    issue()
            else:
                pl.when((unit >= units) if t else (unit < units))(issue)

    def zero_rest(part, parts):
        n = window // ZERO_ROWS // parts

        def issue(c):
            rows = _ds((part * n + c) * ZERO_ROWS, ZERO_ROWS, ZERO_ROWS)
            for t, (grad_hbm, _) in enumerate(grads):
                _start(zero_v.at[pl.ds(0, rest)],
                       grad_hbm.at[pl.ds(n_kv - rest, rest), :, rows], kv_sem.at[t])
        _loop(n, issue, unroll=4)

    def window_rows(which, head, n_heads):
        heads = pl.ds(head, n_heads)

        def issue(c):
            rows = _ds(window + c * DATA_ROWS, DATA_ROWS, DATA_ROWS)
            for t in which:
                grad_hbm, grad_v = grads[t]
                _start(zero_v.at[pl.ds(0, n_heads), 0, pl.ds(0, DATA_ROWS)],
                       grad_hbm.at[heads, 0, rows], kv_sem.at[t])
                _start(grad_v.at[heads, _ds(c * DATA_ROWS, DATA_ROWS, DATA_ROWS)],
                       grad_hbm.at[heads, 1, rows], kv_sem.at[t])
        _loop(window // DATA_ROWS, issue, unroll=8 // len(which))

    def read_everything(sem):
        def read_wq_wo(i):
            rows = _ds(i * 8, 8, 8)
            n = wq_v.shape[2] // CH
            for c in range(n):
                cols = pl.ds(c * CH, CH)
                _start(wq_hbm.at[:, rows, cols], wq_v.at[:, rows, cols], sem.at[2], 0)
                _copy_rows(wo_hbm, wo_v, i * n + c, 8, sem.at[3], 1)

        def read_w3_w4(i):
            rows = _ds(i * 8, 8, 8)
            for c in range(2):
                cols = pl.ds(c * (d_ff // 2), d_ff // 2)
                _start(w3_hbm.at[:, rows, cols], w3_v.at[:, rows, cols], sem.at[4], 0)
                pl.when(i * 2 + c < w4_v.shape[1] // 16)(
                    lambda c=c: _copy_rows(w4_hbm, w4_v, i * 2 + c, 16, sem.at[5], 1))

        def read_kv(lo, n_rows, k_sem, v_sem):
            def group(g):
                heads = pl.ds(g * READ_HEADS, READ_HEADS)

                def chunk(c):
                    src = (heads, _ds(first + lo + c * READ_ROWS, READ_ROWS, READ_ROWS))
                    dst = (heads, _ds(lo + c * READ_ROWS, READ_ROWS, READ_ROWS))
                    _start(k_hbm.at[src], k_v.at[dst], k_sem, 0)
                    _start(v_hbm.at[src], v_v.at[dst], v_sem, 1)
                _loop(n_rows // READ_ROWS, chunk, unroll=5)
            _loop(n_kv // READ_HEADS, group)

        _loop(wq_v.shape[1] // 8, read_wq_wo)
        _start(x_hbm, x_v, sem.at[0], 0)
        _start(go_hbm, go_v, sem.at[1], 1)
        zero_v[...] = jnp.zeros(zero_v.shape, zero_v.dtype)
        o_s[...] = jnp.zeros(o_s.shape, o_s.dtype)
        dq_s[...] = jnp.zeros(dq_s.shape, dq_s.dtype)
        _loop(w3_v.shape[1] // 8, read_w3_w4)
        body = window - TAIL_ROWS
        read_kv(0, body, sem.at[6], sem.at[7])
        read_kv(body, TAIL_ROWS, sem.at[8], sem.at[9])

        for s, ref in enumerate((x_v, go_v, wq_v, wo_v, w3_v, w4_v)):
            _wait(ref, sem.at[s])
        _wait(k_v.at[:, pl.ds(0, body)], sem.at[6])
        _wait(v_v.at[:, pl.ds(0, body)], sem.at[7])
        zero_unit(n_kv // 2, 0, 1)
        _wait(k_v.at[:, pl.ds(body, TAIL_ROWS)], sem.at[8])
        _wait(v_v.at[:, pl.ds(body, TAIL_ROWS)], sem.at[9])

    pl.run_scoped(read_everything, pltpu.SemaphoreType.DMA((10,)))

    pad = jnp.zeros((ROWS - batch, d_model), F32)
    x = jnp.concatenate([x_v[...].astype(F32), pad], axis=0)
    go = jnp.concatenate([go_v[...].astype(F32), pad], axis=0)
    xn, r0 = _layernorm(x)
    u, r1 = _layernorm(xn)
    xn_b = xn.astype(BF16)
    u_b = u.astype(BF16)
    pre = _dot(u_b, w3_v[...].reshape(d_model, d_ff), NN)
    th = jnp.tanh(SQRT_2_OVER_PI * (pre + GELU_C * pre * pre * pre))
    act_b = (0.5 * pre * (1.0 + th)).astype(BF16)
    d_act = 0.5 * (1.0 + th) + (0.5 * pre * (1.0 - th * th) * SQRT_2_OVER_PI
                                * (1.0 + 3.0 * GELU_C * pre * pre))
    y = xn + _dot(act_b, w4_v[...].reshape(d_ff, d_model), NN)
    sig = jax.nn.sigmoid(y)
    gate = y * sig
    ds_b = (go * gate).astype(BF16)

    zero_unit(n_kv // 2 + 1, 0, 2)

    chunk_heads = CH // DH
    n_chunks = HQ // chunk_heads
    wo_chunks = wo_v.shape[1] // CH

    def wq_cols(c):
        return wq_v[:, :, _ds(c * CH, CH, CH)].reshape(d_model, CH)

    def wo_rows(c):
        return lax.div(c, wo_chunks), _ds(lax.rem(c, wo_chunks) * CH, CH, CH)

    def head_rows(c):
        return [_ds((c * chunk_heads + i) * ROWS, ROWS, ROWS) for i in range(chunk_heads)]

    def project(c):
        zero_unit(n_kv // 2 + 1, n_chunks + c, 2 * n_chunks)
        q = _dot(xn_b, wq_cols(c), NN)
        do = _dot(ds_b, wo_v[wo_rows(c)], NT)
        for i, rows in enumerate(head_rows(c)):
            q_s[rows, :] = q[:, i * DH:(i + 1) * DH]
            do_s[rows, :] = do[:, i * DH:(i + 1) * DH]

    _loop(n_chunks, project)

    low = lax.broadcasted_iota(jnp.int32, (2 * rep, 1), 0) < rep

    def attention(i):
        zero_unit(i, 0, 2)
        j = 2 * i
        rows = pl.ds(lax.rem(i, kv_heads // 2) * (2 * rep * ROWS) + lax.div(i, kv_heads // 2),
                     2 * rep, stride=ROWS)

        def pair(lhs, ref, dims):
            return jnp.where(low, _dot(lhs, ref[j], dims), _dot(lhs, ref[j + 1], dims))

        q = q_s[rows, :]
        do = do_s[rows, :]
        s = pair(q.astype(BF16), k_v, NT) * scale
        e = jnp.exp(s - jnp.max(s, axis=-1, keepdims=True))
        p = e * (1.0 / jnp.sum(e, axis=-1, keepdims=True))
        dp = pair(do.astype(BF16), v_v, NT)
        d_s = p * (dp - jnp.sum(p * dp, axis=-1, keepdims=True)) * scale
        o_s[rows, :] = pair(p.astype(BF16), v_v, NN)
        dq_s[rows, :] = pair(d_s.astype(BF16), k_v, NN)
        zero_unit(i, 1, 2)

        lhs = jnp.concatenate([p, d_s], axis=0).astype(BF16)
        z = jnp.zeros((2 * rep, DH), F32)
        rhs = jnp.concatenate([
            jnp.concatenate([jnp.where(low, do, 0.0), jnp.where(low, 0.0, do), z, z], axis=1),
            jnp.concatenate([z, z, jnp.where(low, q, 0.0), jnp.where(low, 0.0, q)], axis=1),
        ], axis=0).astype(BF16)
        for c in range(window // CH):
            keys = pl.ds(c * CH, CH)
            res = _dot(lhs[:, c * CH:(c + 1) * CH], rhs, TN).astype(BF16)
            dv_v[j, keys, :] = res[:, 0:DH]
            dv_v[j + 1, keys, :] = res[:, DH:2 * DH]
            dk_v[j, keys, :] = res[:, 2 * DH:3 * DH]
            dk_v[j + 1, keys, :] = res[:, 3 * DH:4 * DH]

    _loop(n_kv // 2, attention)

    def project_bwd(c, carry):
        attn, dxn = carry
        zero_unit(n_kv // 2 + 2 + lax.div(c, n_chunks // 2), lax.rem(c, n_chunks // 2), n_chunks // 2)
        o_b = jnp.concatenate([o_s[r, :] for r in head_rows(c)], axis=1).astype(BF16)
        dq_b = jnp.concatenate([dq_s[r, :] for r in head_rows(c)], axis=1).astype(BF16)
        attn += _dot(o_b, wo_v[wo_rows(c)], NN)
        dxn += _dot(dq_b, wq_cols(c), NT)
        dwq_v[:, :, _ds(c * CH, CH, CH)] = (
            _dot(xn_b, dq_b, TN).astype(BF16).reshape(dwq_v.shape[0], -1, CH))
        dwo_v[wo_rows(c)] = _dot(o_b, ds_b, TN).astype(BF16)
        return attn, dxn

    acc = jnp.zeros((ROWS, d_model), F32)
    attn, dxn = lax.fori_loop(0, n_chunks, project_bwd, (acc, acc))

    zero_rest(0, 2)

    dy = go * attn * (sig * (1.0 + y * (1.0 - sig)))
    dy_b = dy.astype(BF16)
    dpre_b = (_dot(dy_b, w4_v[...].reshape(d_ff, d_model), NT) * d_act).astype(BF16)
    du = _dot(dpre_b, w3_v[...].reshape(d_model, d_ff), NT)
    dxn = dxn + dy + _layernorm_bwd(u, r1, du)
    out_v[...] = (x + attn * gate)[0:batch].astype(BF16)
    dx_v[...] = (go + _layernorm_bwd(xn, r0, dxn))[0:batch].astype(BF16)

    zero_rest(1, 2)

    ff_slab = dw4_v.shape[1]
    for c in range(dw4_v.shape[0]):
        cols = slice(c * ff_slab, (c + 1) * ff_slab)
        dw3_v[:, :, cols] = (
            _dot(u_b, dpre_b[:, cols], TN).astype(BF16).reshape(dw3_v.shape[0], -1, ff_slab))
        dw4_v[c] = _dot(act_b[:, cols], dy_b, TN).astype(BF16)

    def write_the_rest(sem):
        def write_dwq_dw4(i):
            rows = _ds(i * 8, 8, 8)
            n = dwq_v.shape[2] // (2 * CH)
            for c in range(n):
                cols = pl.ds(c * 2 * CH, 2 * CH)
                _start(dwq_v.at[:, rows, cols], dwq_hbm.at[:, rows, cols], sem.at[2])
                pl.when(i * n + c < dw4_v.shape[1] // 16)(
                    lambda c=c: _copy_rows(dw4_v, dw4_hbm, i * n + c, 16, sem.at[5]))

        def write_dwo_dw3(i):
            rows = _ds(i * 8, 8, 8)
            for c in range(2):
                cols = pl.ds(c * (d_ff // 2), d_ff // 2)
                _copy_rows(dwo_v, dwo_hbm, i * 2 + c, 16, sem.at[3])
                _start(dw3_v.at[:, rows, cols], dw3_hbm.at[:, rows, cols], sem.at[4])

        _start(out_v, out_hbm, sem.at[0])
        _start(dx_v, dx_hbm, sem.at[1])
        _loop(dwq_v.shape[1] // 8, write_dwq_dw4)
        _loop(dw3_v.shape[1] // 8, write_dwo_dw3)
        window_rows((0, 1), n_kv - rest, rest)
        for t in range(2):
            _loop(units, lambda i, t=t: window_rows((t,), i * UNIT_HEADS, UNIT_HEADS))
        for s, ref in enumerate((out_hbm, dx_hbm, dwq_hbm, dwo_hbm, dw3_hbm, dw4_hbm)):
            _wait(ref, sem.at[s])

    pl.run_scoped(write_the_rest, pltpu.SemaphoreType.DMA((6,)))
    _wait(dk_hbm, kv_sem.at[0])
    _wait(dv_hbm, kv_sem.at[1])


@jax.jit
def pallas_recurrent_scan__sliding_block_cached__mixer_s_mlp__decode_kernel(
    A_x: jax.Array,
    A_k_cache: jax.Array,
    A_v_cache: jax.Array,
    A_wq: jax.Array,
    A_wo: jax.Array,
    B_x: jax.Array,
    B_w1: jax.Array,
    B_w2: jax.Array,
    B_w3: jax.Array,
    B_w4: jax.Array,
    grad_out: jax.Array,
):
    del B_x, B_w1, B_w2
    batch, kv_heads, cache_len, _ = A_k_cache.shape
    window = min(4096, max(256, cache_len // 4))
    n_kv = batch * kv_heads
    assert A_x.shape == grad_out.shape == (4, 1, 512)
    assert A_k_cache.shape == A_v_cache.shape == (4, 8, 8192, DH)
    assert A_wq.shape == (512, HQ * DH) and A_wo.shape == (HQ * DH, 512)
    assert B_w3.shape == (512, 1792) and B_w4.shape == (1792, 512)

    def slabs(a, n):
        return a.reshape(n, a.shape[0] // n, a.shape[1])

    x = A_x.reshape(batch, -1)
    go = grad_out.reshape(batch, -1)
    k = A_k_cache.reshape(n_kv, cache_len, DH)
    v = A_v_cache.reshape(n_kv, cache_len, DH)
    wq, wo, w3, w4 = slabs(A_wq, 4), slabs(A_wo, 4), slabs(B_w3, 2), slabs(B_w4, 2)
    dkv = jax.ShapeDtypeStruct((n_kv, 2, cache_len // 2, DH), k.dtype)
    ins = (x, k, v, wq, wo, w3, w4, go)
    outs = (x, x, dkv, dkv, wq, wo, w3, w4)

    def vmem(a):
        return pltpu.VMEM(a.shape, a.dtype)

    hbm = pl.BlockSpec(memory_space=pltpu.HBM)
    win = pltpu.VMEM((n_kv, window, DH), k.dtype)
    heads = pltpu.VMEM(((HQ + 1) * ROWS, DH), F32)
    res = pl.pallas_call(
        _kernel,
        out_shape=[jax.ShapeDtypeStruct(a.shape, a.dtype) for a in outs],
        in_specs=[hbm] * len(ins),
        out_specs=[hbm] * len(outs),
        scratch_shapes=[
            vmem(x), vmem(go), win, win, vmem(wq), vmem(wo), vmem(w3), vmem(w4),
            vmem(x), vmem(x), win, win, vmem(wq), vmem(wo), vmem(w3), vmem(w4),
            pltpu.VMEM((UNIT_HEADS, 2, ZERO_ROWS, DH), k.dtype),
            heads, heads, heads, heads,
            pltpu.SemaphoreType.DMA((2,)),
        ],
        compiler_params=pltpu.CompilerParams(vmem_limit_bytes=110 * 1024 * 1024),
    )(*ins)
    like = (A_x, A_x, A_k_cache, A_v_cache, A_wq, A_wo, B_w3, B_w4)
    return tuple(r.reshape(a.shape) for r, a in zip(res, like))
```

```python
import jax
import jax.numpy as jnp
from jax import lax
import jax.experimental.pallas as pl
import jax.experimental.pallas.tpu as pltpu

F32 = jnp.float32
BF16 = jnp.bfloat16

HQ = 32
DH = 128
EPS = 1e-5
SQRT_2_OVER_PI = 0.7978845608028654
GELU_C = 0.044715

ROWS = 8
CH = 512
READ_HEADS = 8
READ_ROWS = 16
TAIL_ROWS = 48
UNIT_HEADS = 3
FINE_ROWS = 16
COARSE_ROWS = 64

NN = (((1,), (0,)), ((), ()))
NT = (((1,), (1,)), ((), ()))
TN = (((0,), (0,)), ((), ()))


def _dot(a, b, dims):
    return lax.dot_general(a, b, dims, preferred_element_type=F32)


def _layernorm(x):
    xc = x - jnp.mean(x, axis=-1, keepdims=True)
    r = 1.0 / jnp.sqrt(jnp.mean(xc * xc, axis=-1, keepdims=True) + EPS)
    return xc * r, r


def _layernorm_bwd(y, r, dy):
    return r * (dy - jnp.mean(dy, axis=-1, keepdims=True)
                - y * jnp.mean(dy * y, axis=-1, keepdims=True))


def _loop(n, body, unroll=1):
    unroll = min(unroll, n)
    assert n % unroll == 0, (n, unroll)
    if n == unroll:
        for u in range(n):
            body(u)
        return

    def step(i, carry):
        for u in range(unroll):
            body(i * unroll + u)
        return carry

    lax.fori_loop(0, n // unroll, step, 0)


def _ds(start, size, align):
    if not isinstance(start, int):
        start = pl.multiple_of(start, align)
    return pl.ds(start, size)


def _start(src, dst, sem, priority=0):
    pltpu.make_async_copy(src, dst, sem).start(priority=priority)


def _wait(ref, sem):
    pltpu.make_async_copy(ref, ref, sem).wait()


def _copy_rows(src, dst, i, rows, sem, priority=0):
    r = _ds(i * rows, rows, rows)
    _start(src.at[:, r], dst.at[:, r], sem, priority)


def _kernel(x_hbm, k_hbm, v_hbm, wq_hbm, wo_hbm, w3_hbm, w4_hbm, go_hbm,
            out_hbm, dx_hbm, dk_hbm, dv_hbm, dwq_hbm, dwo_hbm, dw3_hbm, dw4_hbm,
            x_v, go_v, k_v, v_v, wq_v, wo_v, w3_v, w4_v,
            out_v, dx_v, dk_v, dv_v, dwq_v, dwo_v, dw3_v, dw4_v,
            zero_fine, zero_coarse, q_s, do_s, o_s, dq_s, kv_sem):
    batch, d_model = x_v.shape
    n_kv, window, _ = k_v.shape
    kv_heads = n_kv // batch
    first = k_hbm.shape[1] - window
    d_ff = w3_v.shape[2]
    rep = HQ // kv_heads
    scale = DH ** -0.5
    grads = ((dk_hbm, dk_v), (dv_hbm, dv_v))
    units = (n_kv - 5) // UNIT_HEADS
    fives = (((n_kv - 5, 3), (n_kv - 5, 2)), ((n_kv - 2, 2), (n_kv - 3, 3)))

    def zero_unit(unit, part, parts, zeros):
        height = zeros.shape[2]
        n = window // height // parts
        for t, (grad_hbm, _) in enumerate(grads):
            def issue(t=t, grad_hbm=grad_hbm):
                heads = pl.ds((unit - t * units) * UNIT_HEADS, UNIT_HEADS)
                _loop(n, lambda c: _start(
                    zeros, grad_hbm.at[heads, :, _ds((part * n + c) * height, height, height)],
                    kv_sem.at[t]), unroll=8)
            if isinstance(unit, int):
                if unit // units == t:
                    issue()
            else:
                pl.when((unit >= units) if t else (unit < units))(issue)

    def zero_five(t, group, part, parts):
        n = window // COARSE_ROWS // parts

        def issue(c):
            rows = _ds((part * n + c) * COARSE_ROWS, COARSE_ROWS, COARSE_ROWS)
            for half, (head, count) in enumerate(group):
                _start(zero_coarse.at[pl.ds(0, count), 0],
                       grads[t][0].at[pl.ds(head, count), half, rows], kv_sem.at[t])
        _loop(n, issue, unroll=4)

    def window_rows(t, group, zeros):
        grad_hbm, grad_v = grads[t]
        low, high = group
        height = zeros.shape[2]

        def issue(c):
            rows = _ds(window + c * height, height, height)
            _start(zeros.at[pl.ds(0, low[1]), 0],
                   grad_hbm.at[pl.ds(*low), 0, rows], kv_sem.at[t])
            _start(grad_v.at[pl.ds(*high), _ds(c * height, height, height)],
                   grad_hbm.at[pl.ds(*high), 1, rows], kv_sem.at[t])
        _loop(window // height, issue, unroll=8)

    def read_everything(sem):
        def read_wq_wo(i):
            rows = _ds(i * 8, 8, 8)
            n = wq_v.shape[2] // CH
            for c in range(n):
                cols = pl.ds(c * CH, CH)
                _start(wq_hbm.at[:, rows, cols], wq_v.at[:, rows, cols], sem.at[2], 0)
                _copy_rows(wo_hbm, wo_v, i * n + c, 8, sem.at[3], 1)

        def read_w3_w4(i):
            rows = _ds(i * 8, 8, 8)
            for c in range(2):
                cols = pl.ds(c * (d_ff // 2), d_ff // 2)
                _start(w3_hbm.at[:, rows, cols], w3_v.at[:, rows, cols], sem.at[4], 0)
                pl.when(i * 2 + c < w4_v.shape[1] // 16)(
                    lambda c=c: _copy_rows(w4_hbm, w4_v, i * 2 + c, 16, sem.at[5], 1))

        def read_kv(lo, n_rows, k_sem, v_sem):
            def group(g):
                heads = pl.ds(g * READ_HEADS, READ_HEADS)

                def chunk(c):
                    src = (heads, _ds(first + lo + c * READ_ROWS, READ_ROWS, READ_ROWS))
                    dst = (heads, _ds(lo + c * READ_ROWS, READ_ROWS, READ_ROWS))
                    _start(k_hbm.at[src], k_v.at[dst], k_sem, 0)
                    _start(v_hbm.at[src], v_v.at[dst], v_sem, 1)
                _loop(n_rows // READ_ROWS, chunk, unroll=5)
            _loop(n_kv // READ_HEADS, group)

        _loop(wq_v.shape[1] // 8, read_wq_wo)
        _start(x_hbm, x_v, sem.at[0], 0)
        _start(go_hbm, go_v, sem.at[1], 1)
        for ref in (zero_fine, zero_coarse, o_s, dq_s):
            ref[...] = jnp.zeros(ref.shape, ref.dtype)
        _loop(w3_v.shape[1] // 8, read_w3_w4)
        body = window - TAIL_ROWS
        read_kv(0, body, sem.at[6], sem.at[7])
        read_kv(body, TAIL_ROWS, sem.at[8], sem.at[9])

        for s, ref in enumerate((x_v, go_v, wq_v, wo_v, w3_v, w4_v)):
            _wait(ref, sem.at[s])
        _wait(k_v.at[:, pl.ds(0, body)], sem.at[6])
        _wait(v_v.at[:, pl.ds(0, body)], sem.at[7])
        zero_unit(n_kv // 2, 0, 1, zero_coarse)
        _wait(k_v.at[:, pl.ds(body, TAIL_ROWS)], sem.at[8])
        _wait(v_v.at[:, pl.ds(body, TAIL_ROWS)], sem.at[9])

    pl.run_scoped(read_everything, pltpu.SemaphoreType.DMA((10,)))

    pad = jnp.zeros((ROWS - batch, d_model), F32)
    x = jnp.concatenate([x_v[...].astype(F32), pad], axis=0)
    go = jnp.concatenate([go_v[...].astype(F32), pad], axis=0)
    xn, r0 = _layernorm(x)
    u, r1 = _layernorm(xn)
    xn_b = xn.astype(BF16)
    u_b = u.astype(BF16)
    pre = _dot(u_b, w3_v[...].reshape(d_model, d_ff), NN)
    th = jnp.tanh(SQRT_2_OVER_PI * (pre + GELU_C * pre * pre * pre))
    act_b = (0.5 * pre * (1.0 + th)).astype(BF16)
    d_act = 0.5 * (1.0 + th) + (0.5 * pre * (1.0 - th * th) * SQRT_2_OVER_PI
                                * (1.0 + 3.0 * GELU_C * pre * pre))
    y = xn + _dot(act_b, w4_v[...].reshape(d_ff, d_model), NN)
    sig = jax.nn.sigmoid(y)
    gate = y * sig
    ds_b = (go * gate).astype(BF16)

    zero_unit(n_kv // 2 + 1, 0, 2, zero_coarse)

    chunk_heads = CH // DH
    n_chunks = HQ // chunk_heads
    wo_chunks = wo_v.shape[1] // CH

    def wq_cols(c):
        return wq_v[:, :, _ds(c * CH, CH, CH)].reshape(d_model, CH)

    def wo_rows(c):
        return lax.div(c, wo_chunks), _ds(lax.rem(c, wo_chunks) * CH, CH, CH)

    def head_rows(c):
        return [_ds((c * chunk_heads + i) * ROWS, ROWS, ROWS) for i in range(chunk_heads)]

    def project(c):
        zero_unit(n_kv // 2 + 1, n_chunks + c, 2 * n_chunks, zero_coarse)
        q = _dot(xn_b, wq_cols(c), NN)
        do = _dot(ds_b, wo_v[wo_rows(c)], NT)
        for i, rows in enumerate(head_rows(c)):
            q_s[rows, :] = q[:, i * DH:(i + 1) * DH]
            do_s[rows, :] = do[:, i * DH:(i + 1) * DH]

    _loop(n_chunks, project)

    low = lax.broadcasted_iota(jnp.int32, (2 * rep, 1), 0) < rep

    def attention(i):
        zero_unit(i, 0, 4, zero_fine)
        j = 2 * i
        rows = pl.ds(lax.rem(i, kv_heads // 2) * (2 * rep * ROWS) + lax.div(i, kv_heads // 2),
                     2 * rep, stride=ROWS)

        def pair(lhs, ref, dims):
            return jnp.where(low, _dot(lhs, ref[j], dims), _dot(lhs, ref[j + 1], dims))

        q = q_s[rows, :]
        do = do_s[rows, :]
        s = pair(q.astype(BF16), k_v, NT) * scale
        e = jnp.exp(s - jnp.max(s, axis=-1, keepdims=True))
        p = e * (1.0 / jnp.sum(e, axis=-1, keepdims=True))
        dp = pair(do.astype(BF16), v_v, NT)
        d_s = p * (dp - jnp.sum(p * dp, axis=-1, keepdims=True)) * scale
        zero_unit(i, 1, 4, zero_fine)
        o_s[rows, :] = pair(p.astype(BF16), v_v, NN)
        dq_s[rows, :] = pair(d_s.astype(BF16), k_v, NN)
        zero_unit(i, 2, 4, zero_fine)

        lhs = jnp.concatenate([p, d_s], axis=0).astype(BF16)
        z = jnp.zeros((2 * rep, DH), F32)
        rhs = jnp.concatenate([
            jnp.concatenate([jnp.where(low, do, 0.0), jnp.where(low, 0.0, do), z, z], axis=1),
            jnp.concatenate([z, z, jnp.where(low, q, 0.0), jnp.where(low, 0.0, q)], axis=1),
        ], axis=0).astype(BF16)
        for c in range(window // CH):
            if c == window // CH // 2:
                zero_unit(i, 3, 4, zero_fine)
            keys = pl.ds(c * CH, CH)
            res = _dot(lhs[:, c * CH:(c + 1) * CH], rhs, TN).astype(BF16)
            dv_v[j, keys, :] = res[:, 0:DH]
            dv_v[j + 1, keys, :] = res[:, DH:2 * DH]
            dk_v[j, keys, :] = res[:, 2 * DH:3 * DH]
            dk_v[j + 1, keys, :] = res[:, 3 * DH:4 * DH]

    _loop(n_kv // 2, attention)

    def project_bwd(c, carry):
        attn, dxn = carry
        parts = n_chunks // 4
        for g in range(4):
            pl.when(lax.div(c, parts) == g)(
                lambda g=g: zero_five(g // 2, fives[g % 2], lax.rem(c, parts), parts))
        o_b = jnp.concatenate([o_s[r, :] for r in head_rows(c)], axis=1).astype(BF16)
        dq_b = jnp.concatenate([dq_s[r, :] for r in head_rows(c)], axis=1).astype(BF16)
        attn += _dot(o_b, wo_v[wo_rows(c)], NN)
        dxn += _dot(dq_b, wq_cols(c), NT)
        dwq_v[:, :, _ds(c * CH, CH, CH)] = (
            _dot(xn_b, dq_b, TN).astype(BF16).reshape(dwq_v.shape[0], -1, CH))
        dwo_v[wo_rows(c)] = _dot(o_b, ds_b, TN).astype(BF16)
        return attn, dxn

    acc = jnp.zeros((ROWS, d_model), F32)
    attn, dxn = lax.fori_loop(0, n_chunks, project_bwd, (acc, acc))

    window_rows(0, fives[0], zero_coarse)

    dy = go * attn * (sig * (1.0 + y * (1.0 - sig)))
    dy_b = dy.astype(BF16)
    dpre_b = (_dot(dy_b, w4_v[...].reshape(d_ff, d_model), NT) * d_act).astype(BF16)
    du = _dot(dpre_b, w3_v[...].reshape(d_model, d_ff), NT)
    dxn = dxn + dy + _layernorm_bwd(u, r1, du)
    out_v[...] = (x + attn * gate)[0:batch].astype(BF16)
    dx_v[...] = (go + _layernorm_bwd(xn, r0, dxn))[0:batch].astype(BF16)

    window_rows(0, fives[1], zero_coarse)

    ff_slab = dw4_v.shape[1]
    for c in range(dw4_v.shape[0]):
        cols = slice(c * ff_slab, (c + 1) * ff_slab)
        dw3_v[:, :, cols] = (
            _dot(u_b, dpre_b[:, cols], TN).astype(BF16).reshape(dw3_v.shape[0], -1, ff_slab))
        dw4_v[c] = _dot(act_b[:, cols], dy_b, TN).astype(BF16)

    def write_the_rest(sem):
        def write_dwq_dw4(i):
            rows = _ds(i * 8, 8, 8)
            n = dwq_v.shape[2] // (2 * CH)
            for c in range(n):
                cols = pl.ds(c * 2 * CH, 2 * CH)
                _start(dwq_v.at[:, rows, cols], dwq_hbm.at[:, rows, cols], sem.at[2])
                pl.when(i * n + c < dw4_v.shape[1] // 16)(
                    lambda c=c: _copy_rows(dw4_v, dw4_hbm, i * n + c, 16, sem.at[5]))

        def write_dwo_dw3(i):
            rows = _ds(i * 8, 8, 8)
            for c in range(2):
                cols = pl.ds(c * (d_ff // 2), d_ff // 2)
                _copy_rows(dwo_v, dwo_hbm, i * 2 + c, 16, sem.at[3])
                _start(dw3_v.at[:, rows, cols], dw3_hbm.at[:, rows, cols], sem.at[4])

        def write_units(t):
            _loop(units, lambda i: window_rows(t, ((i * UNIT_HEADS, UNIT_HEADS),) * 2, zero_fine))

        write_units(0)
        _start(out_v, out_hbm, sem.at[0])
        _start(dx_v, dx_hbm, sem.at[1])
        _loop(dwq_v.shape[1] // 8, write_dwq_dw4)
        _loop(dw3_v.shape[1] // 8, write_dwo_dw3)
        write_units(1)
        for group in fives:
            window_rows(1, group, zero_fine)
        for s, ref in enumerate((out_hbm, dx_hbm, dwq_hbm, dwo_hbm, dw3_hbm, dw4_hbm)):
            _wait(ref, sem.at[s])

    pl.run_scoped(write_the_rest, pltpu.SemaphoreType.DMA((6,)))
    _wait(dk_hbm, kv_sem.at[0])
    _wait(dv_hbm, kv_sem.at[1])


@jax.jit
def pallas_recurrent_scan__sliding_block_cached__mixer_s_mlp__decode_kernel(
    A_x: jax.Array,
    A_k_cache: jax.Array,
    A_v_cache: jax.Array,
    A_wq: jax.Array,
    A_wo: jax.Array,
    B_x: jax.Array,
    B_w1: jax.Array,
    B_w2: jax.Array,
    B_w3: jax.Array,
    B_w4: jax.Array,
    grad_out: jax.Array,
):
    del B_x, B_w1, B_w2
    batch, kv_heads, cache_len, _ = A_k_cache.shape
    window = min(4096, max(256, cache_len // 4))
    n_kv = batch * kv_heads
    assert A_x.shape == grad_out.shape == (4, 1, 512)
    assert A_k_cache.shape == A_v_cache.shape == (4, 8, 8192, DH)
    assert A_wq.shape == (512, HQ * DH) and A_wo.shape == (HQ * DH, 512)
    assert B_w3.shape == (512, 1792) and B_w4.shape == (1792, 512)

    def slabs(a, n):
        return a.reshape(n, a.shape[0] // n, a.shape[1])

    x = A_x.reshape(batch, -1)
    go = grad_out.reshape(batch, -1)
    k = A_k_cache.reshape(n_kv, cache_len, DH)
    v = A_v_cache.reshape(n_kv, cache_len, DH)
    wq, wo, w3, w4 = slabs(A_wq, 4), slabs(A_wo, 4), slabs(B_w3, 2), slabs(B_w4, 2)
    dkv = jax.ShapeDtypeStruct((n_kv, 2, cache_len // 2, DH), k.dtype)
    ins = (x, k, v, wq, wo, w3, w4, go)
    outs = (x, x, dkv, dkv, wq, wo, w3, w4)

    def vmem(a):
        return pltpu.VMEM(a.shape, a.dtype)

    hbm = pl.BlockSpec(memory_space=pltpu.HBM)
    win = pltpu.VMEM((n_kv, window, DH), k.dtype)
    heads = pltpu.VMEM(((HQ + 1) * ROWS, DH), F32)
    res = pl.pallas_call(
        _kernel,
        out_shape=[jax.ShapeDtypeStruct(a.shape, a.dtype) for a in outs],
        in_specs=[hbm] * len(ins),
        out_specs=[hbm] * len(outs),
        scratch_shapes=[
            vmem(x), vmem(go), win, win, vmem(wq), vmem(wo), vmem(w3), vmem(w4),
            vmem(x), vmem(x), win, win, vmem(wq), vmem(wo), vmem(w3), vmem(w4),
            pltpu.VMEM((UNIT_HEADS, 2, FINE_ROWS, DH), k.dtype),
            pltpu.VMEM((UNIT_HEADS, 2, COARSE_ROWS, DH), k.dtype),
            heads, heads, heads, heads,
            pltpu.SemaphoreType.DMA((2,)),
        ],
        compiler_params=pltpu.CompilerParams(vmem_limit_bytes=110 * 1024 * 1024),
    )(*ins)
    like = (A_x, A_x, A_k_cache, A_v_cache, A_wq, A_wo, B_w3, B_w4)
    return tuple(r.reshape(a.shape) for r, a in zip(res, like))
```
